```python
import os as _os
_os.environ.setdefault('JAX_PLATFORMS', 'cpu')
import jax
import jax.numpy as jnp

def _softmax(x, axis=-1):
    return jax.nn.softmax(x, axis=axis)

def _gelu(x):
    return jax.nn.gelu(x, approximate=True)

def _silu(x):
    return jax.nn.silu(x)

def _sigmoid(x):
    return jax.nn.sigmoid(x)

def _layernorm(x, axis=-1, eps=1e-05):
    m = jnp.mean(x, axis=axis, keepdims=True)
    v = jnp.var(x, axis=axis, keepdims=True)
    return (x - m) / jnp.sqrt(v + eps)

def _scatter_add(tgt, idx, src, axis=0):
    return tgt.at[idx].add(src)

def _segment_sum(src, seg, n):
    return jax.ops.segment_sum(src, seg, n)

class _Rng:

    def __init__(self, key):
        self._k = key

    def _next(self):
        self._k, sub = jax.random.split(self._k)
        return sub

    def normal(self, shape):
        return jax.random.normal(self._next(), shape, dtype=jnp.bfloat16)

    def randint(self, lo, hi, shape):
        return jax.random.randint(self._next(), shape, lo, hi, dtype=jnp.int32)

    def uniform(self, shape, lo=0.0, hi=1.0):
        return jax.random.uniform(self._next(), shape, jnp.bfloat16, lo, hi)

    def permutation(self, n):
        return jax.random.permutation(self._next(), n)
kernel_name = 'adaLN_cond__grouped_kv_mqa__mixer_gmlp__prompt'

def setup_inputs():
    _rng = _Rng(jax.random.key(int.from_bytes(__import__("os").urandom(4), "little")))
    _w = lambda a: (lambda t: t.astype(jnp.bfloat16) if jnp.issubdtype(t.dtype, jnp.floating) else t)(jnp.asarray(a))

    def _A_setup():
        B, S, D, H = (1, 2048, 512, 32)
        Dh = D // H
        return {'x': _w((lambda *s: _rng.normal(s) * 0.05)(B, S, D)), 'wq': _w((lambda *s: _rng.normal(s) * 0.05)(D, H * Dh)), 'wk': _w((lambda *s: _rng.normal(s) * 0.05)(D, Dh)), 'wv': _w((lambda *s: _rng.normal(s) * 0.05)(D, Dh)), 'wo': _w((lambda *s: _rng.normal(s) * 0.05)(H * Dh, D))}
    _A_in = _A_setup()

    def _B_setup():
        B, S, D, F = (1, 2048, 512, 1792)
        Fh = F // 2
        return {'x': _w((lambda *s: _rng.normal(s) * 0.05)(B, S, D)), 'w_in': _w((lambda *s: _rng.normal(s) * 0.4)(D, 2 * Fh)), 'w_sp': _w(0.01 * (lambda *s: _rng.normal(s) * 0.4)(S, S)), 'b_sp': _w(1.0 + 0.01 * (lambda *s: _rng.normal(s) * 0.05)(S)), 'w_out': _w((lambda *s: _rng.normal(s) * 0.05)(Fh, D))}
    _B_in = _B_setup()
    return {'A_x': _A_in['x'], 'A_wq': _A_in['wq'], 'A_wk': _A_in['wk'], 'A_wv': _A_in['wv'], 'A_wo': _A_in['wo'], 'B_x': _B_in['x'], 'B_w_in': _B_in['w_in'], 'B_w_sp': _B_in['w_sp'], 'B_b_sp': _B_in['b_sp'], 'B_w_out': _B_in['w_out'], 'c': _w((lambda *s: _rng.normal(s) * 0.05)(1, 512) * 8.0), 'w_mod': _w((lambda *s: _rng.normal(s) * 0.05)(512, 6 * 512) * 512 ** (-0.5) * 8.0)}

def reference(A_x, A_wq, A_wk, A_wv, A_wo, B_x, B_w_in, B_w_sp, B_b_sp, B_w_out, c, w_mod):

    def _A_ref(x, wq, wk, wv, wo):
        B, S, D = x.shape
        H = 32
        Dh = D // H
        q = (lambda x, *d: x.transpose(*d))((x @ wq).reshape(B, S, H, Dh), 0, 2, 1, 3)
        k = x @ wk
        v = x @ wv
        scores = jnp.einsum('bhqd,bkd->bhqk', q, k) * Dh ** (-0.5)
        p = _softmax(scores, axis=-1)
        o = jnp.einsum('bhqk,bkd->bhqd', p, v)
        return (lambda x, *d: x.transpose(*d))(o, 0, 2, 1, 3).reshape(B, S, H * Dh) @ wo

    def _B_ref(x, w_in, w_sp, b_sp, w_out):
        B, S, D = x.shape
        F = w_in.shape[-1]
        Fh = F // 2
        z = _gelu(jnp.einsum('bsd,df->bsf', x, w_in))
        z1 = z[..., :Fh].copy()
        z2 = _layernorm(z[..., Fh:], axis=-1)
        g = jnp.einsum('ts,bsf->btf', w_sp, z2) + b_sp[None, :, None]
        return jnp.einsum('bsf,fd->bsd', z1 * g, w_out)
    x = A_x
    mod = (_silu(c) @ w_mod).reshape(c.shape[0], 6, 1, -1)
    sa, ca, ga, sb, cb, gb = (mod[:, 0].copy(), mod[:, 1].copy(), mod[:, 2].copy(), mod[:, 3].copy(), mod[:, 4].copy(), mod[:, 5].copy())
    h = _layernorm(x, axis=-1) * (1 + ca) + sa
    x = x + ga * _A_ref(h, A_wq, A_wk, A_wv, A_wo)
    h = _layernorm(x, axis=-1) * (1 + cb) + sb
    x = x + gb * _B_ref(h, B_w_in, B_w_sp, B_b_sp, B_w_out)
    return x
```

```python
import functools
import math

import jax
import jax.numpy as jnp
from jax import lax
import jax.experimental.pallas as pl
import jax.experimental.pallas.tpu as pltpu

CFG = dict(un=4, lag=1, win=10, nvp=16, forcesafe=0, scopes=0, rbc=256, rbd=256)

S, D, H, DH, F, FH = 2048, 512, 32, 16, 1792, 896
QB = 512
KC = 128
NC = S // KC
NU = (S // QB) * H
SV0 = S // 2
EPS = 1e-5
QSCALE = DH ** -0.5 * math.log2(math.e)
L_MIN, L_MAX = 2.0 ** -40, 2.0 ** 40

bf16, f32, u32 = jnp.bfloat16, jnp.float32, jnp.uint32
NN = (((1,), (0,)), ((), ()))
NT = (((1,), (1,)), ((), ()))


def _dot(a, b, dims=NN):
    return lax.dot_general(a, b, dims, preferred_element_type=f32)


def _layernorm(x):
    m = jnp.mean(x, axis=-1, keepdims=True)
    xc = x - m
    v = jnp.mean(xc * xc, axis=-1, keepdims=True)
    return xc * lax.rsqrt(v + EPS)


def _gelu(x):
    c = math.sqrt(2.0 / math.pi)
    inner = x * (c + (c * 0.044715) * (x * x))
    hx = 0.5 * x
    return hx + hx * jnp.tanh(inner)


class _Scope:
    def __init__(self, name):
        self.cm = jax.named_scope(name) if CFG['scopes'] else None

    def __enter__(self):
        if self.cm is not None:
            self.cm.__enter__()

    def __exit__(self, *a):
        if self.cm is not None:
            self.cm.__exit__(*a)


def _kernel(x_hbm, wq_hbm, wkt_hbm, wvt_hbm, wo_hbm, win_hbm, wsp_hbm, bsp_hbm, wout_hbm, c_hbm, wmod_hbm,
            o_hbm,
            x_v, wq_v, wo_v, win_v, wsp_v, bsp_v, wout_v, c_v, wmod_v,
            mod_v, wt_v, qs_v, qf_v, ks_v, kn_v, vs_v, kb_v, p_v, ot_v, s_v,
            x1_v, z1_v, z2_v, bcol_v, out_v, sem, xsem, osem):
    UN, LAG, WIN, NVP = CFG['un'], CFG['lag'], CFG['win'], CFG['nvp']
    RBC, RBD = CFG['rbc'], CFG['rbd']
    nblk = S // QB

    def cp(src, dst, i):
        return pltpu.make_async_copy(src, dst, sem.at[i])

    c_cp = cp(c_hbm, c_v, 0)
    wmod_a_cp = cp(wmod_hbm.at[:, pl.ds(0, 2 * D)], wmod_v.at[:, pl.ds(0, 2 * D)], 1)
    wq_cp = cp(wq_hbm, wq_v, 2)
    wk_cp = cp(wkt_hbm, wt_v.at[pl.ds(D, DH), :], 3)
    wv_cp = cp(wvt_hbm, wt_v.at[pl.ds(D + DH, DH), :], 4)
    wmod_b_cp = cp(wmod_hbm.at[:, pl.ds(2 * D, 4 * D)], wmod_v.at[:, pl.ds(2 * D, 4 * D)], 5)
    wo_cp = cp(wo_hbm, wo_v, 6)
    win_cp = cp(win_hbm, win_v, 7)
    wsp_cp = cp(wsp_hbm, wsp_v, 8)
    bsp_cp = cp(bsp_hbm, bsp_v, 9)
    wout_cp = cp(wout_hbm, wout_v, 10)

    def x_cp(i):
        r = pl.ds(pl.multiple_of(i * QB, QB), QB)
        return pltpu.make_async_copy(x_hbm.at[r, :], x_v.at[r, :], xsem.at[i])

    for c_ in (c_cp, wq_cp, wk_cp, wv_cp, wmod_a_cp):
        c_.start()
    for i in range(nblk):
        x_cp(i).start()

    with _Scope("A0"):
        wq_cp.wait()
        wt_v[pl.ds(0, D), :] = wq_v[...].astype(f32).T.astype(bf16)
        wk_cp.wait()
        wv_cp.wait()
        c_cp.wait()
        cf = c_v[...].astype(f32)
        sc = jnp.broadcast_to(cf * jax.nn.sigmoid(cf), (16, D)).astype(bf16)
        wmod_a_cp.wait()
        mod_v[:, pl.ds(0, 2 * D)] = _dot(sc, wmod_v[:, pl.ds(0, 2 * D)])[:8]

    npj = [((j + 1) * NVP) // NC - (j * NVP) // NC for j in range(NC)]
    pidx = [sum(npj[:j]) for j in range(NC)]
    cpb = QB // KC
    assert all(npj[j] == npj[j % cpb] for j in range(NC))
    ppb = sum(npj[:cpb])

    def vpu_groups(j):
        return list(range(8 - npj[j], 8))

    def mxu_groups(j):
        return [g for g in range(8) if g not in vpu_groups(j)][::-1]

    def qkv_block(i, carry):
        x_cp(i).wait()
        r = pl.ds(pl.multiple_of(i * QB, QB), QB)
        shift, scale = mod_v[0:1, pl.ds(0, D)], mod_v[0:1, pl.ds(D, D)]
        h = (_layernorm(x_v[r, :].astype(f32)) * (1.0 + scale) + shift).astype(bf16)
        t = _dot(wt_v[...], h, NT)
        q = (t[:D] * QSCALE).astype(bf16)
        for hh in range(H):
            qh = q[hh * DH:(hh + 1) * DH]
            qs_v[i * H + hh] = pltpu.bitcast(qh, u32)
            qf_v[i * H + hh] = qh.astype(f32)
        vt = t[D + DH:].astype(bf16)
        for jj in range(cpb):
            vs_v[i * cpb + jj] = pltpu.bitcast(vt[:, jj * KC:(jj + 1) * KC], u32)
        kf = t[D:D + DH].astype(bf16).astype(f32).T
        kn_v[r, :] = kf.astype(bf16)
        for jj in range(cpb):
            for n, g in enumerate(mxu_groups(jj)):
                row = pl.multiple_of(i * (QB // 2) + jj * 64 + n * 8, 8)
                kg = kf[jj * KC + g * 16:jj * KC + (g + 1) * 16]
                ks_v[pl.ds(row, 8), pl.ds(0, DH)] = pltpu.bitcast(kg.astype(bf16), u32)
            for n, g in enumerate(vpu_groups(jj)):
                kg = kf[jj * KC + g * 16:jj * KC + (g + 1) * 16]
                for d in range(DH):
                    kb_v[i * ppb + pidx[jj] + n, d] = jnp.broadcast_to(kg[:, d:d + 1], (16, 128))
        return carry

    with _Scope("A1"):
        lax.fori_loop(0, nblk, qkv_block, 0)

    for c_ in (wmod_b_cp, wo_cp, win_cp, bsp_cp, wout_cp, wsp_cp):
        c_.start()

    def svrow(pi, t, c):
        return SV0 + ((pi * 4 + c) * 2 + t) * 8

    def vpu_stream(units, z):
        for u, pis in units:
            for pi in pis:
                for c in range(4):
                    accs = [None, None]
                    for d in range(DH):
                        qb = jnp.broadcast_to(qf_v[u, pl.ds(d, 1), pl.ds(c * 128, 128)], (8, 128))
                        for t in range(2):
                            pr = kb_v[pi, d, pl.ds(t * 8, 8), :] * qb
                            accs[t] = pr if d == 0 else accs[t] + pr
                    for t in range(2):
                        row = z + svrow(pi, t, c)
                        if not isinstance(row, int):
                            row = pl.multiple_of(row, 8)
                        ks_v[pl.ds(row, 8), :] = pltpu.bitcast(accs[t], u32)
                    yield

    def qk(u, j, l, adv, marks):
        svs = {}
        for n, g in enumerate(vpu_groups(j)):
            pi = pidx[j] + n
            svs[g] = jnp.concatenate(
                [jnp.concatenate([pltpu.bitcast(ks_v[pl.ds(svrow(pi, t, c), 8), :], f32) for t in range(2)], axis=0)
                 for c in range(4)], axis=1)
        q = pltpu.bitcast(qs_v[u], bf16)
        ks = []
        for n, g in enumerate(mxu_groups(j)):
            adv()
            ks.append(ks_v[pl.ds(j * 64 + n * 8, 8), pl.ds(0, DH)])
        s = _dot(pltpu.bitcast(jnp.concatenate(ks, axis=0), bf16), q)
        for n, g in enumerate(mxu_groups(j)):
            svs[g] = s[n * 16:(n + 1) * 16]
            marks.append(s[n * 16:n * 16 + 8, :128])
        pg = [None] * 8
        for g in reversed(range(8)):
            p = jnp.exp2(svs[g])
            l = p[:8] + p[8:] if l is None else l + p[:8] + p[8:]
            pg[g] = p
        return jnp.concatenate(pg, axis=0).astype(bf16), l

    def pv(j, ptile, acc):
        o = _dot(pltpu.bitcast(vs_v[j], bf16), ptile)
        return o if acc is None else acc + o

    def fin(u, acc, l, bad):
        den = jnp.sum(l, axis=0, keepdims=True)
        o = acc * (1.0 / den)
        ot_v[u] = o
        ok = jnp.logical_and(jnp.logical_and(den >= L_MIN, den <= L_MAX),
                             jnp.maximum(jnp.abs(o[:8]), jnp.abs(o[8:])) < jnp.inf)
        return jnp.where(ok, bad, 1.0)

    nlead = min(NVP, 1)
    total_groups = NC * 8 - NVP

    def attn_body(it, carry):
        acc, l_prev, bad = carry
        z = jnp.minimum(it, 0)
        units = [(it * UN + uu, range(nlead if uu == 0 else 0, NVP)) for uu in range(UN)]
        units.append((jnp.minimum(it * UN + UN, NU - 1), range(nlead)))
        gen = vpu_stream(units, z)
        marks = []
        state = dict(done=0, groups=0)

        def adv():
            state['groups'] += 1
            target = (state['groups'] * NVP * 4) // total_groups
            while state['done'] < target:
                mi = min(state['groups'] - 1 - WIN, len(marks) - 1)
                if mi >= 0:
                    qf_v[z + NU, pl.ds(0, 8), pl.ds(0, 128)] = marks[mi]
                next(gen)
                state['done'] += 1

        held = {}
        for uu in range(UN):
            u = it * UN + uu
            l = None
            for j in range(NC):
                pt, l = qk(u, j, l, adv, marks)
                if uu == UN - 1 and j >= NC - LAG:
                    p_v[j - (NC - LAG)] = pt
                else:
                    held[uu, j] = pt
                if j < LAG:
                    jj = NC - LAG + j
                    acc = pv(jj, held.pop((uu - 1, jj)) if uu else p_v[j], acc)
                    if j == LAG - 1:
                        bad = fin(jnp.maximum(u - 1, 0), acc, l_prev, bad)
                        acc = None
                else:
                    acc = pv(j - LAG, held.pop((uu, j - LAG)), acc)
            l_prev = l
        return acc, l_prev, bad

    with _Scope("B"):
        for j in range(LAG):
            p_v[j] = jnp.zeros((KC, QB), bf16)
        for _ in vpu_stream([(0, range(nlead))], 0):
            pass
        carry = (jnp.zeros((DH, QB), f32), jnp.ones((8, QB), f32), jnp.zeros((8, QB), f32))
        acc, l, bad = lax.fori_loop(0, NU // UN, attn_body, carry)
        for j in range(LAG):
            acc = pv(NC - LAG + j, p_v[j], acc)
        bad = fin(NU - 1, acc, l, bad)
        unsafe = jnp.max(bad) > 0.0
        if CFG['forcesafe']:
            unsafe = jnp.max(bad) > -1.0

    @pl.when(unsafe)
    def _():
        def safe_unit(u, carry):
            q = pltpu.bitcast(qs_v[u], bf16)

            def scores(j, m):
                r = pl.ds(pl.multiple_of(j * KC, KC), KC)
                s = _dot(kn_v[r, :], q)
                s_v[r, :] = s
                return jnp.maximum(m, jnp.max(s, axis=0, keepdims=True))

            m = lax.fori_loop(0, NC, scores, jnp.full((1, QB), -jnp.inf, f32))

            def weighted(j, c):
                acc_, l_ = c
                r = pl.ds(pl.multiple_of(j * KC, KC), KC)
                p = jnp.exp2(s_v[r, :] - m)
                return (acc_ + _dot(pltpu.bitcast(vs_v[j], bf16), p.astype(bf16)),
                        l_ + jnp.sum(p, axis=0, keepdims=True))

            acc_, l_ = lax.fori_loop(0, NC, weighted, (jnp.zeros((DH, QB), f32), jnp.zeros((1, QB), f32)))
            ot_v[u] = acc_ * (1.0 / l_)
            return carry

        lax.fori_loop(0, NU, safe_unit, 0)

    with _Scope("C0"):
        wmod_b_cp.wait()
        mod_v[:, pl.ds(2 * D, 4 * D)] = _dot(sc, wmod_v[:, pl.ds(2 * D, 4 * D)])[:8]
        bsp_cp.wait()
        bf = bsp_v[...].astype(f32)
        for j in range(S // 128):
            bcol_v[pl.ds(j * 128, 128), :] = jnp.broadcast_to(bf[j:j + 1, :], (128, 128)).T
        wo_cp.wait()
        win_cp.wait()

    def mlp_in_block(i, carry):
        ga = mod_v[0:1, pl.ds(2 * D, D)]
        sb, cb = mod_v[0:1, pl.ds(3 * D, D)], mod_v[0:1, pl.ds(4 * D, D)]
        ot = ot_v[pl.ds(i * H, H)].reshape(D, QB)
        hs = []
        for a in range(QB // RBC):
            r = pl.ds(pl.multiple_of(i * QB + a * RBC, RBC), RBC)
            o = ot[:, a * RBC:(a + 1) * RBC].T.astype(bf16)
            x1 = x_v[r, :].astype(f32) + ga * _dot(o, wo_v[...])
            x1_v[r, :] = x1
            hs.append((_layernorm(x1) * (1.0 + cb) + sb).astype(bf16))
        for a in range(QB // RBC):
            r = pl.ds(pl.multiple_of(i * QB + a * RBC, RBC), RBC)
            z2 = _gelu(_dot(hs[a], win_v[:, pl.ds(FH, FH)]))
            z2_v[r, :] = _layernorm(z2).astype(bf16)
        for a in range(QB // RBC):
            r = pl.ds(pl.multiple_of(i * QB + a * RBC, RBC), RBC)
            z1_v[r, :] = _gelu(_dot(hs[a], win_v[:, pl.ds(0, FH)]))
        return carry

    with _Scope("C1"):
        lax.fori_loop(0, nblk, mlp_in_block, 0)

    wsp_cp.wait()
    wout_cp.wait()

    def o_cp(i):
        r = pl.ds(pl.multiple_of(i * QB, QB), QB)
        return pltpu.make_async_copy(out_v.at[r, :], o_hbm.at[r, :], osem.at[i])

    def mlp_out_block(i, carry):
        gb = mod_v[0:1, pl.ds(5 * D, D)]
        ys = []
        for a in range(QB // RBD):
            r = pl.ds(pl.multiple_of(i * QB + a * RBD, RBD), RBD)
            g = _dot(wsp_v[r, :], z2_v[...]) + jnp.concatenate([bcol_v[r, :]] * (FH // 128), axis=1)
            ys.append((z1_v[r, :] * g).astype(bf16))
        for a in range(QB // RBD):
            r = pl.ds(pl.multiple_of(i * QB + a * RBD, RBD), RBD)
            out_v[r, :] = (x1_v[r, :] + gb * _dot(ys[a], wout_v[...])).astype(bf16)
        o_cp(i).start()
        return carry

    with _Scope("D"):
        lax.fori_loop(0, nblk, mlp_out_block, 0)
        for i in range(nblk):
            o_cp(i).wait()


@jax.jit
def pallas_adaLN_cond__grouped_kv_mqa__mixer_gmlp__prompt_kernel(
        A_x, A_wq, A_wk, A_wv, A_wo, B_x, B_w_in, B_w_sp, B_b_sp, B_w_out, c, w_mod):
    del B_x
    nvp, lag = max(CFG['nvp'], 1), CFG['lag']
    vm = pltpu.VMEM
    scratch = [
        vm((S, D), bf16), vm((D, D), bf16), vm((D, D), bf16),
        vm((D, F), bf16), vm((S, S), bf16), vm((S // 128, 128), bf16), vm((FH, D), bf16),
        vm((1, D), bf16), vm((D, 6 * D), bf16),
        vm((8, 6 * D), f32),
        vm((D + 2 * DH, D), bf16),
        vm((NU, DH // 2, QB), u32),
        vm((NU + 1, DH, QB), f32),
        vm((SV0 + nvp * 64, 128), u32),
        vm((S, DH), bf16),
        vm((NC, DH // 2, KC), u32),
        vm((nvp, DH, 16, 128), f32),
        vm((lag, KC, QB), bf16),
        vm((NU, DH, QB), f32),
        vm((S, QB), f32),
        vm((S, D), f32),
        vm((S, FH), f32),
        vm((S, FH), bf16),
        vm((S, 128), f32),
        vm((S, D), bf16),
        pltpu.SemaphoreType.DMA((11,)), pltpu.SemaphoreType.DMA((S // QB,)), pltpu.SemaphoreType.DMA((S // QB,)),
    ]
    out = pl.pallas_call(
        _kernel,
        out_shape=jax.ShapeDtypeStruct((S, D), bf16),
        in_specs=[pl.BlockSpec(memory_space=pl.ANY)] * 11,
        out_specs=pl.BlockSpec(memory_space=pl.ANY),
        scratch_shapes=scratch,
        compiler_params=pltpu.CompilerParams(vmem_limit_bytes=110 * 2 ** 20),
    )(A_x.reshape(S, D), A_wq, A_wk.T, A_wv.T, A_wo, B_w_in, B_w_sp, B_b_sp.reshape(S // 128, 128), B_w_out, c, w_mod)
    return out.reshape(1, S, D)
```

```python
import functools
import math

import jax
import jax.numpy as jnp
from jax import lax
import jax.experimental.pallas as pl
import jax.experimental.pallas.tpu as pltpu

S, D, H, DH, FH = 2048, 512, 32, 16, 896
HS, HD = S // 2, D // 2
EPS = 1e-5
QSCALE = DH ** -0.5 * math.log2(math.e)

QB = 512
KC = 128
NC = S // KC
NU = (S // QB) * H
UNROLL = 8
NVG = 22
LEAD = 4
Q_AHEAD = 9
STEPS, GROUPS = 44, 53
STEP_DUE = (1, 2, 4, 5, 6, 7, 8, 8, 9, 11, 13, 14, 15, 16, 18, 19, 20, 21, 22, 24, 25, 26, 27, 28, 30,
            31, 32, 33, 35, 35, 37, 39, 39, 40, 42, 43, 44, 45, 47, 48, 49, 50, 52, 52)
STEP_START = ((11, 11, 10, 13, 13, 12, 12, 9, 13, 11, 11, 12, 11, 12, 11, 10, 12, 10, 11, 8, 10, 13, 11,
               5, 11, 11, 11, 10, 11, 13, 11, 10, 11, 10, 11, 8, 10, 10, 11, 9, 11, 10, 11, 8),
              (9, 10, 10, 11, 10, 10, 10, 9, 10, 10, 10, 11, 11, 10, 10, 10, 10, 9, 9, 10, 10, 10, 10,
               10, 12, 10, 10, 10, 11, 10, 10, 10, 12, 18, 12, 10, 16, 11, 10, 11, 10, 11, 10, 9))
PV_DELAY = (1, 3, 2, 1, 3, 1, 2, 1)
DEN_MIN, DEN_MAX, V_MAX = 2.0 ** -80, 2.0 ** 97, 2.0 ** 20

_NV = [((j + 2) * NVG) // NC - ((j + 1) * NVG) // NC for j in range(NC)]
VPU_GROUPS = [list(range(8 - n, 8)) for n in _NV]
MXU_GROUPS = [list(range(8 - n))[::-1] for n in _NV]
VPU_FIRST = [sum(_NV[:j]) for j in range(NC)]
STREAM = [(j, g) for j in range(NC) for g in MXU_GROUPS[j]]
NG = len(STREAM)
STREAM_END = [sum(len(g) for g in MXU_GROUPS[:j + 1]) for j in range(NC)]
SV0 = S // 2
X_SPLIT = (0, 2, 4, 8, NC)

RB = 256
NSTEP = HS // RB
FS = 384
MIXED = (0, 2, 3, 5, 6)

PACING = ((672, -256, 416), (416, 640, 352), (608, 128, 384), (608, 128, 320), (384, 448, 352),
          (608, 384, 320), (768, -192, 416), (256, 384, 448), (576, 128, 320),
          (480, -64, 256), (608, 128, 448), (544, 128, 416), (800, 64, 448))
REST_FIRST = (1, 2, 1, 2, 0, 1, 2, 2)
INNER_FIRST = ((5, 7, 4, 0), (7, 5, 4, 0), (7, 4, 0, 6), (7, 4, 0), (4, 7, 1, 0, 6), (6, 7, 4), (7, 4, 0))

bf16, f32, u32 = jnp.bfloat16, jnp.float32, jnp.uint32
NN = (((1,), (0,)), ((), ()))
NT = (((1,), (1,)), ((), ()))


def _dot(a, b, dims=NN):
    return lax.dot_general(a, b, dims, preferred_element_type=f32)


def _rows(start, size):
    return pl.ds(start if isinstance(start, int) else pl.multiple_of(start, size), size)


def _layernorm(x, eps=EPS, scale=1.0):
    m = jnp.mean(x, axis=-1, keepdims=True)
    xc = x - m
    r = lax.rsqrt(jnp.mean(xc * xc, axis=-1, keepdims=True) + eps)
    return xc * (r if scale == 1.0 else r * scale)


def _gelu2(x):
    c = math.sqrt(2.0 / math.pi)
    return x + x * jnp.tanh(x * (c + (c * 0.044715) * (x * x)))


def _strassen_lhs(a11, a12, a21, a22):
    f11, f12, f21, f22 = (a.astype(f32) for a in (a11, a12, a21, a22))
    return f11 + f22, f21 + f22, a11, a22, f11 + f12, f21 - f11, f12 - f22


def _strassen_rhs(b11, b12, b21, b22):
    f11, f12, f21, f22 = (b.astype(f32) for b in (b11, b12, b21, b22))
    return f11 + f22, b11, f12 - f22, f21 - f11, b22, f11 + f12, f21 + f22


def _strassen(product, done=lambda i, j, c: None):
    m3 = product(2)
    m5 = product(4)
    c12 = m3 + m5
    done(0, 1, c12)
    m1 = product(0)
    m2 = product(1)
    c22 = product(5) + ((m1 - m2) + m3)
    done(1, 1, c22)
    m4 = product(3)
    c21 = m2 + m4
    done(1, 0, c21)
    c11 = product(6) + ((m1 + m4) - m5)
    done(0, 0, c11)
    return c11, c12, c21, c22


def _winograd_lhs(a11, a12, a21, a22):
    s1 = a21 + a22
    s2 = s1 - a11
    return a11, a12, a12 - s2, a22, s1, s2, a11 - a21


def _winograd_rhs(b11, b12, b21, b22):
    t1 = b12 - b11
    t2 = b22 - t1
    return b11, b21, b22, t2 - b21, t1, t2, b22 - b12


class _Pacer:
    def __init__(self):
        self.free, self.turn = [0] * 4, 0
        self.marks, self.pending = [], []

    def add(self, items, start_gate, first, last, window, tag):
        now = min(self.free)
        for n, item in enumerate(items):
            due = now + first + (last - first) * n // (len(items) - 1)
            self.pending.append((due, item, start_gate, tag, window))
        self.pending.sort(key=lambda e: e[0])

    def dot(self, lhs, rhs):
        start = self.free[self.turn % 4]
        head, tied = lhs[:8, :128], False
        while self.pending and self.pending[0][0] <= start:
            due, item, start_gate, _, window = self.pending.pop(0)
            ready = [v for t, v in self.marks if t <= due - window]
            if ready and start_gate is not None:
                start_gate(ready[-1])
            head, tied = jnp.minimum(head, jnp.maximum(head, item())), True
        if tied:
            lhs = jnp.concatenate([jnp.concatenate([head, lhs[:8, 128:]], axis=1), lhs[8:]], axis=0)
        out = _dot(lhs, rhs)
        (m, k), n = lhs.shape, rhs.shape[1]
        for _ in range((k // 128) * (n // 128)):
            last = self.free[self.turn % 4]
            self.free[self.turn % 4] += m
            self.turn += 1
        for r in range(0, m, 64):
            self.marks.append((last + r + 133, out[r:r + 8, n - 128:]))
        self.marks.sort(key=lambda e: e[0])
        return out

    def flush(self, tag=None):
        due = [e for e in self.pending if tag is None or e[3] == tag]
        self.pending = [e for e in self.pending if not (tag is None or e[3] == tag)]
        for entry in due:
            entry[1]()


def _kernel(x_hbm, wq_hbm, wkt_hbm, wvt_hbm, wo_hbm, win_hbm, wsp_hbm, bsp_hbm, wout_hbm, c_hbm, wmod_hbm,
            o_hbm,
            x_v, wq_v, wo_v, win_v, wsp_v, wout_v, wmod_v, mod_v, wkv_v, wl_v,
            qa_v, qc0_v, qc1_v, acc_v, den_v, ks_v, vs_v, kb_v, p_v, ot_v, lt_v, s_v,
            l0_v, l1_v, l2_v, l3_v, wc_v, atta_v, attb_v, ua_v, ub_v,
            x1_v, z1_v, z2_v, bcol_v, out_v, bsp_v, c_v, sem, xsem, osem):

    def copy(src, dst, i):
        return pltpu.make_async_copy(src, dst, sem.at[i])

    def x_cp(i):
        r = pl.ds(X_SPLIT[i] * KC, (X_SPLIT[i + 1] - X_SPLIT[i]) * KC)
        return pltpu.make_async_copy(x_hbm.at[r, :], x_v.at[r, :], xsem.at[i])

    c_cp = copy(c_hbm, c_v.at[:, pl.ds(0, D)], 0)
    wmod_cp = copy(wmod_hbm.at[:, pl.ds(0, 2 * D)], wmod_v.at[:, pl.ds(0, 2 * D)], 1)
    wq_cp = copy(wq_hbm, wq_v, 2)
    wk_cp = copy(wkt_hbm, wkv_v.at[pl.ds(0, DH), :], 3)
    wv_cp = copy(wvt_hbm, wkv_v.at[pl.ds(DH, DH), :], 4)
    late_cps = (copy(wmod_hbm.at[:, pl.ds(2 * D, 4 * D)], wmod_v.at[:, pl.ds(2 * D, 4 * D)], 5),
                copy(wo_hbm, wo_v, 6), copy(win_hbm, win_v, 7), copy(bsp_hbm, bsp_v, 9),
                copy(wout_hbm, wout_v, 10), copy(wsp_hbm, wsp_v, 8))

    for cp in (c_cp, wk_cp, wv_cp, wq_cp):
        cp.start()
    c_cp.wait()
    x_cp(0).start()
    wk_cp.wait()
    wmod_cp.start()
    wv_cp.wait()
    x_cp(1).start()
    cf = c_v[:, pl.ds(0, D)].astype(f32)
    silu_c = jnp.broadcast_to(cf * jax.nn.sigmoid(cf), (16, D)).astype(bf16)
    wq_cp.wait()
    x_cp(2).start()
    wqt = wq_v[...].astype(f32).T
    for k, v in enumerate(_strassen_lhs(wqt[:HD, :HD], wqt[:HD, HD:], wqt[HD:, :HD], wqt[HD:, HD:])):
        wl_v[k] = v
    x_cp(0).wait()
    x_cp(3).start()
    first = pl.ds(0, X_SPLIT[1] * KC)
    x1_v[first, :] = _layernorm(x_v[first, :].astype(f32))
    wmod_cp.wait()
    mod_a = _dot(silu_c, wmod_v[:, pl.ds(0, 2 * D)])
    shift_a, scale_a = mod_a[0:1, :D], 1.0 + mod_a[0:1, D:]

    hs, vpu_keys, v_max = [], [], jnp.zeros((8, KC), f32)
    for j0 in range(0, NC, 2):
        for j in range(len(hs), min(j0 + 4, NC)):
            if j in X_SPLIT[1:]:
                x_cp(X_SPLIT.index(j)).wait()
            r = pl.ds(j * KC, KC)
            xn = x1_v[r, :] if j < X_SPLIT[1] else _layernorm(x_v[r, :].astype(f32))
            hs.append(xn * scale_a + shift_a)
        for j in (j0, j0 + 1):
            kv = _dot(wkv_v[...], hs[j], NT)
            vs_v[j] = pltpu.bitcast(kv[DH:].astype(bf16), u32)
            v_max = jnp.maximum(v_max, jnp.maximum(jnp.abs(kv[DH:DH + 8]), jnp.abs(kv[DH + 8:])))
            keys = kv[:DH].T
            ks_v[pl.ds(j * (KC // 2), KC // 2), pl.ds(0, DH)] = pltpu.bitcast(keys.astype(bf16), u32)
            vpu_keys.extend((VPU_FIRST[j] + n, keys[g * 16:(g + 1) * 16]) for n, g in enumerate(VPU_GROUPS[j]))
        h0, h1 = hs[j0], hs[j0 + 1]
        h_ops = _strassen_rhs(h0[:, :HD], h1[:, :HD], h0[:, HD:], h1[:, HD:])

        def q_product(k):
            if k != 6:
                return _dot(wl_v[k], h_ops[k], NT)
            return jnp.concatenate([_dot(wl_v[k, pl.ds(a * HD // 2, HD // 2), :], h_ops[k], NT)
                                    for a in range(2)], axis=0)

        def put_q(a, b, qt):
            j = j0 + b
            for n in range(H // 2):
                qa_v[(j * KC // QB) * H + a * (H // 2) + n, :, pl.ds(j * KC % QB, KC)] = (
                    qt[n * DH:(n + 1) * DH] * QSCALE)

        _strassen(q_product, put_q)
        if len(hs) == NC:
            keys = jnp.concatenate([v for _, v in vpu_keys], axis=0)
            for d in range(DH // 2):
                lo, hi = (jnp.broadcast_to(keys[:, e:e + 1], (keys.shape[0], 128)) for e in (d, d + DH // 2))
                for n, (slot, _) in enumerate(vpu_keys):
                    r0, r1 = slice(n * 16, n * 16 + 8), slice(n * 16 + 8, n * 16 + 16)
                    for k, v in enumerate(_winograd_lhs(lo[r0], hi[r0], lo[r1], hi[r1])):
                        kb_v[slot // 2, k, d, pl.ds((slot % 2) * 8, 8), :] = v
            vpu_keys = []

    def sv_row(slot, t, c):
        return SV0 + (((slot // 2) * 2 + t) * 4 + c) * 16 + (slot % 2) * 8

    def q_operands(u, side):
        for cp in range(2):
            q0, q1 = (qa_v[u, :, pl.ds(cp * 256 + c * 128, 128)] for c in range(2))
            for k, v in enumerate(_winograd_rhs(q0[:8], q1[:8], q0[8:], q1[8:])):
                for qc_v in (qc0_v, qc1_v):
                    qc_v[side, :, pl.ds((cp * 7 + k) * 128, 128)] = v
                yield

    def vpu_scores(units, zero, gates):
        count, upcoming = 0, iter(())
        for u_next, side, pairs in units:
            for pair in pairs:
                if u_next is not None and pair == Q_AHEAD:
                    upcoming = q_operands(u_next, 1 - side)
                for cp in range(2):
                    def product(k, half):
                        qc_v = (qc0_v, qc1_v)[count % 2]
                        if gates and gates[half] is not None:
                            qc_v[zero + 2, :, pl.ds(0, 128)] = gates[half]
                        for d in range(8):
                            row = qc_v[side, pl.ds(d, 1), pl.ds((cp * 7 + k) * 128, 128)]
                            term = kb_v[pair, k, d] * jnp.broadcast_to(row, (16, 128))
                            m = term if d == 0 else m + term
                        return m

                    def park(t, c, block):
                        ks_v[_rows(zero + sv_row(2 * pair, t, 2 * cp + c), 16), :] = pltpu.bitcast(block, u32)

                    def steps():
                        p1 = product(0, 0)
                        park(0, 0, p1 + product(1, 1))
                        yield
                        u2 = p1 + product(5, 0)
                        u3 = u2 + product(6, 1)
                        park(1, 1, u3)
                        yield
                        p5 = product(4, 0)
                        park(1, 0, u3 - product(3, 1))
                        park(1, 1, u3 + p5)
                        u4 = u2 + p5
                        yield
                        park(0, 1, u4 + product(2, 1))
                        yield

                    for _ in steps():
                        count += 1
                        next(upcoming, None)
                        next(upcoming, None)
                        yield

    def add_pv(j, pt, zero):
        o = _dot(pltpu.bitcast(vs_v[j], bf16), pt)
        if j:
            o = o + acc_v[zero]
        if j < NC - 1:
            acc_v[zero] = o
        return o

    def put_o(u, o, lsum):
        for half in range(QB // RB):
            cols = slice(half * RB, (half + 1) * RB)
            ot_v[(u // H) * (QB // RB) + half, u % H] = o[:, cols]
            lt_v[(u // H) * (QB // RB) + half, u % H] = lsum[:, cols]

    def finish_unit(u, o, lsum):
        put_o(u, o, lsum)
        lo, hi = den_v[0], den_v[1]
        for c in range(QB // 128):
            lo = jnp.minimum(lo, lsum[:, c * 128:(c + 1) * 128])
            hi = jnp.maximum(hi, lsum[:, c * 128:(c + 1) * 128])
        den_v[0], den_v[1] = lo, hi

    def softmax_items(i):
        def item(b, n):
            heads = pl.ds(n, 4)
            den = jnp.sum(lt_v[b, heads], axis=1, keepdims=True)
            r = pltpu.reciprocal(den, approx=True)
            o = ot_v[b, heads] * (r * (2.0 - den * r))
            ot_v[b, heads] = o
            return o[3, :8, 128:]

        return [functools.partial(item, i + a * NSTEP, n) for a in range(2) for n in range(0, H, 4)]

    def attention_step(it, l_prev):
        zero = jnp.minimum(it, 0)
        units = [(jnp.minimum(it * UNROLL + n + 1, NU - 1), n % 2, range(LEAD // 2 if n == 0 else 0, NVG // 2))
                 for n in range(UNROLL)]
        units.append((None, 0, range(LEAD // 2)))
        gates, marks, scores = [], [], {}
        vpu_steps = vpu_scores(units, zero, gates)
        progress = [0]

        def mxu_scores(lo, hi):
            while lo < hi:
                n = lo // NG
                end = min(hi, (n + 1) * NG)
                q = qa_v[it * UNROLL + n]
                keys = []
                for pos in range(lo, end):
                    while (pos >= 4 and progress[0] < UNROLL * NVG * 4
                           and progress[0] // STEPS * GROUPS + STEP_DUE[progress[0] % STEPS] <= pos):
                        at = [min(pos - w[progress[0] % STEPS], len(marks) - 1) for w in STEP_START]
                        gates[:] = [marks[a] if a >= 0 else None for a in at]
                        next(vpu_steps)
                        progress[0] += 1
                    j, g = STREAM[pos - n * NG]
                    keys.append(ks_v[pl.ds(j * 64 + g * 8, 8), pl.ds(0, DH)])
                s = _dot(pltpu.bitcast(jnp.concatenate(keys, axis=0), bf16), q)
                for pos in range(lo, end):
                    scores[(n,) + STREAM[pos - n * NG]] = s[(pos - lo) * 16:(pos - lo + 1) * 16]
                    marks.append(s[(pos - lo) * 16:(pos - lo) * 16 + 8, 0:128])
                lo = end

        def probabilities(n, j, lsum):
            for i, g in enumerate(VPU_GROUPS[j]):
                slot = VPU_FIRST[j] + i
                assert progress[0] >= (n * NVG + slot // 2 * 2 + 2 - LEAD) * 4
                scores[n, j, g] = jnp.concatenate([jnp.concatenate(
                    [pltpu.bitcast(ks_v[pl.ds(sv_row(slot, t, c), 8), :], f32) for t in range(2)], axis=0)
                    for c in range(QB // 128)], axis=1)
            pt = [None] * 8
            for g in reversed(range(8)):
                p = pt[g] = jnp.exp2(scores.pop((n, j, g)))
                lsum = p[:8] + p[8:] if lsum is None else lsum + p[:8] + p[8:]
            return jnp.concatenate(pt, axis=0), lsum

        pos, prev = 0, p_v[...]
        for n in range(UNROLL):
            lsum = None
            for j in range(NC):
                end = min(n * NG + STREAM_END[j] + PV_DELAY[j % len(PV_DELAY)], UNROLL * NG)
                mxu_scores(pos, end)
                pos = end
                pt, lsum = probabilities(n, j, lsum)
                if j == 0:
                    finish_unit(jnp.maximum(it * UNROLL + n - 1, 0), add_pv(NC - 1, prev, zero), l_prev)
                else:
                    add_pv(j - 1, prev, zero)
                prev = pt
            l_prev = lsum
        p_v[...] = prev
        for _ in vpu_steps:
            pass
        return l_prev

    for cp in late_cps:
        cp.start()
    p_v[...] = jnp.zeros((KC, QB), f32)
    for _ in q_operands(0, 0):
        pass
    for _ in vpu_scores([(None, 0, range(LEAD // 2))], 0, []):
        pass
    acc_v[0] = jnp.zeros((DH, QB), f32)
    den_v[0] = den_v[1] = jnp.ones((8, 128), f32)
    den_v[2] = v_max
    lsum = lax.fori_loop(0, NU // UNROLL, attention_step, jnp.ones((8, QB), f32))
    for cp in late_cps:
        cp.wait()
    finish_unit(NU - 1, add_pv(NC - 1, p_v[...], 0), lsum)

    for item in softmax_items(0):
        item()
    mod_v[:, pl.ds(2 * D, 4 * D)] = _dot(silu_c, wmod_v[:, pl.ds(2 * D, 4 * D)])[:8]
    safe = jnp.logical_and(jnp.logical_and(den_v[0] >= DEN_MIN, den_v[1] <= DEN_MAX), den_v[2] <= V_MAX)
    unsafe = jnp.max(jnp.where(safe, 0, 1))
    zero = jnp.minimum(unsafe, 0)

    @pl.when(unsafe > 0)
    def _():
        def unit(u, carry):
            q = qa_v[u]

            def score_chunk(j, m):
                keys = ks_v[_rows(j * (KC // 2), KC // 2), pl.ds(0, DH)]
                s = _dot(pltpu.bitcast(keys, bf16), q)
                s_v[_rows(j * KC, KC), :] = s
                return jnp.maximum(m, jnp.max(s, axis=0, keepdims=True))

            m = lax.fori_loop(0, NC, score_chunk, jnp.full((1, QB), -jnp.inf, f32))

            def value_chunk(j, sums):
                p = jnp.exp2(s_v[_rows(j * KC, KC), :] - m)
                return (sums[0] + _dot(pltpu.bitcast(vs_v[j], bf16), p),
                        sums[1] + jnp.sum(p, axis=0, keepdims=True))

            o, den = lax.fori_loop(0, NC, value_chunk, (jnp.zeros((DH, QB), f32), jnp.zeros((1, QB), f32)))
            put_o(u, o * (1.0 / den), jnp.full((8, QB), 0.125, f32))
            return carry

        lax.fori_loop(0, NU, unit, 0)

    l_v, att_v, u_v = (l0_v, l1_v, l2_v, l3_v), (atta_v, attb_v), (ua_v, ub_v)
    pacer = _Pacer()

    def gate(src_v):
        def start_gate(v):
            src_v[_rows(zero + 2 * RB, 8), pl.ds(0, 128)] = v
        return start_gate

    def attn_out(i):
        for a in range(2):
            o = ot_v[i + a * NSTEP].reshape(D, RB).T
            for n in range(0, D, 128):
                att_v[i % 2][pl.ds(a * RB, RB), pl.ds(n, 128)] = pacer.dot(o, wo_v[:, pl.ds(n, 128)])

    def weight_items():
        def item(p, n):
            lo, hi = pl.ds(p * FH, FS), pl.ds(p * FH + FS, FS)
            r0, r1 = pl.ds(n, 16), pl.ds(HD + n, 16)
            ops = _strassen_rhs(win_v[r0, lo], win_v[r0, hi], win_v[r1, lo], win_v[r1, hi])
            for m, k in enumerate(MIXED):
                wc_v[p * len(MIXED) + m, r0, :] = ops[k]
            return ops[0][:8, :128]

        return [functools.partial(item, p, n) for p in (1, 0) for n in range(0, HD, 16)]

    def norm1_items(i):
        gate_a = mod_v[0:1, pl.ds(2 * D, D)]
        shift_b, scale_b = mod_v[0:1, pl.ds(3 * D, D)], 1.0 + mod_v[0:1, pl.ds(4 * D, D)]

        def item(n):
            h = []
            for a in range(2):
                row = a * HS + i * RB + n
                x = x_v[pl.ds(row - n % 16, 16), :].astype(f32)[n % 16:n % 16 + 8]
                x1 = x + gate_a * att_v[i % 2][_rows(zero + a * RB + n, 8), :]
                x1_v[pl.ds(row, 8), :] = x1
                h.append(_layernorm(x1) * scale_b + shift_b)
            ops = _strassen_lhs(h[0][:, :HD], h[0][:, HD:], h[1][:, :HD], h[1][:, HD:])
            for k, v in enumerate(ops + (h[0][:, HD:], h[1][:, :HD])):
                l_v[i][k, pl.ds(n, 8), :] = v
            return ops[0][:, :128]

        return [functools.partial(item, n) for n in range(0, RB, 8)]

    def norm2_items(i):
        def item(a, n):
            z2 = _layernorm(_gelu2(u_v[i % 2][_rows(zero + a * RB + n, 8), :]), 4.0 * EPS, 0.5)
            z2_v[pl.ds(a * HS + i * RB + n, 8), :] = z2
            return z2[:, :128]

        return [functools.partial(item, a, n) for a in range(2) for n in range(0, RB, 8)]

    def bias_items():
        def item(j):
            col = jnp.broadcast_to(0.5 * bsp_v[...].astype(f32)[j:j + 1, :], (128, 128)).T
            bcol_v[pl.ds(j * 128, 128), :] = col
            return col[:8]

        return [functools.partial(item, j) for j in range(S // 128)]

    def project(i, p):
        blocks = []
        for n in range(0, FS, 128):
            ops = [None] * 7
            for m, k in enumerate(MIXED):
                ops[k] = wc_v[p * len(MIXED) + m, :, pl.ds(n, 128)]
            ops[1] = win_v[pl.ds(0, HD), pl.ds(p * FH + n, 128)]
            ops[4] = win_v[pl.ds(HD, HD), pl.ds(p * FH + FS + n, 128)]
            blocks.append(ops)

        def rest_columns(a):
            k0, k1 = ((2, 7), (8, 3))[a]
            return pacer.dot(jnp.concatenate([l_v[i][k0], l_v[i][k1]], axis=1),
                             win_v[:, pl.ds(p * FH + 2 * FS, FH - 2 * FS)])

        def block(ops):
            early = {k: pacer.dot(l_v[i][k], ops[k]) for k in (2, 4, 0)}
            return _strassen(lambda k: early[k] if k in early else pacer.dot(l_v[i][k], ops[k]))

        rests = [rest_columns(a) for a in range(REST_FIRST[2 * i + p])]
        blocks = [block(ops) for ops in blocks]
        for a in range(2):
            rest = rests[a] if a < len(rests) else rest_columns(a)
            blocks.append(jnp.concatenate([b[2 * a] for b in blocks[:3]] + [b[2 * a + 1] for b in blocks[:3]]
                                          + [rest], axis=1))
        for a in range(2):
            if p:
                u_v[i % 2][pl.ds(a * RB, RB), :] = blocks[3 + a]
            else:
                z1_v[pl.ds(a * HS + i * RB, RB), :] = blocks[3 + a]

    t_out, t_proj = 32 * RB // 4, 50 * RB // 4
    pacing = list(PACING)

    def pace(items, start_gate, span, tag=None):
        first, margin, window = pacing.pop(0)
        pacer.add(items, start_gate, first, span - margin, window, tag)

    pace(weight_items(), None, t_out)
    pace(softmax_items(1), None, t_out, 3)
    attn_out(0)
    pacer.flush(3)
    pace(norm1_items(0), gate(att_v[0]), t_out)
    attn_out(1)
    pacer.flush()
    for i in range(NSTEP):
        ahead = t_out if i + 2 < NSTEP else 0
        if i + 1 < NSTEP:
            pace(norm1_items(i + 1), gate(att_v[(i + 1) % 2]), 2 * t_proj + ahead, 1)
        else:
            pace(bias_items(), None, t_proj)
        if ahead:
            pace(softmax_items(i + 2), None, 2 * t_proj, 3)
        project(i, 1)
        pacer.flush(2)
        pace(norm2_items(i), gate(u_v[i % 2]), t_proj + ahead + (t_proj if i + 1 < NSTEP else 0), 2)
        project(i, 0)
        if ahead:
            pacer.flush(3)
            attn_out(i + 2)
        pacer.flush(1)
    pacer.flush()

    hr, hk = RB // 2, HS // 2

    def quarter(i, q):
        return _rows(q * (S // 4) + i * hr, hr)

    def o_cp(i, q, b):
        r, c = quarter(i, q), pl.ds(b * HD, HD)
        return pltpu.make_async_copy(out_v.at[r, c], o_hbm.at[r, c], osem.at[8 * i + 2 * q + b])

    def gating_step(i, carry):
        gate_b = mod_v[0:1, pl.ds(5 * D, D)]
        lo, hi = pl.ds(0, HS), pl.ds(HS, HS)

        def rows(ref, a, cols=slice(None)):
            return jnp.concatenate([ref[quarter(i, 2 * a + e), cols] for e in range(2)], axis=0)

        def product(k):
            w = _strassen_lhs(rows(wsp_v, 0, lo), rows(wsp_v, 0, hi), rows(wsp_v, 1, lo), rows(wsp_v, 1, hi))[k]
            z = _strassen_rhs(z2_v[lo, pl.ds(0, FS)], z2_v[lo, pl.ds(FS, FS)],
                              z2_v[hi, pl.ds(0, FS)], z2_v[hi, pl.ds(FS, FS)])[k]
            w_ops = _strassen_lhs(w[:hr, :hk], w[:hr, hk:], w[hr:, :hk], w[hr:, hk:])
            z_ops = _strassen_rhs(z[:hk, :128], z[:hk, 128:256], z[hk:, :128], z[hk:, 128:256])
            early = {m: _dot(w_ops[m], z_ops[m]) if m < 7 else _dot(w, z[:, 256:]) for m in INNER_FIRST[k]}
            c11, c12, c21, c22 = _strassen(lambda m: early[m] if m in early else _dot(w_ops[m], z_ops[m]))
            inner = jnp.concatenate([jnp.concatenate([c11, c12], axis=1),
                                     jnp.concatenate([c21, c22], axis=1)], axis=0)
            return jnp.concatenate([inner, early[7]], axis=1)

        def rest_columns(a):
            return _dot(rows(wsp_v, a), z2_v[:, pl.ds(2 * FS, FH - 2 * FS)])

        g_rest = [rest_columns(0)]
        g_early = {k: product(k) for k in (3, 1)}
        g_blocks = _strassen(lambda k: g_early[k] if k in g_early else product(k))
        g_rest.append(rest_columns(1))
        ys = []
        for a in range(2):
            g = jnp.concatenate([g_blocks[2 * a], g_blocks[2 * a + 1], g_rest[a]], axis=1)
            g = g + jnp.concatenate([rows(bcol_v, a)] * (FH // 128), axis=1)
            ys.append(_gelu2(rows(z1_v, a)) * g)
        o_rest = [_dot(y[:, 2 * FS:], wout_v[pl.ds(2 * FS, FH - 2 * FS), :]) for y in ys]

        def put_out(a, b, block):
            c = slice(b * HD, (b + 1) * HD)
            out = rows(x1_v, a, pl.ds(b * HD, HD)) + gate_b[:, c] * (block + o_rest[a][:, c])
            for e in range(2):
                out_v[quarter(i, 2 * a + e), pl.ds(b * HD, HD)] = out[e * hr:(e + 1) * hr].astype(bf16)
                o_cp(i, 2 * a + e, b).start()

        w_ops = _strassen_rhs(wout_v[pl.ds(0, FS), pl.ds(0, HD)], wout_v[pl.ds(0, FS), pl.ds(HD, HD)],
                              wout_v[pl.ds(FS, FS), pl.ds(0, HD)], wout_v[pl.ds(FS, FS), pl.ds(HD, HD)])
        y_ops = _strassen_lhs(ys[0][:, :FS], ys[0][:, FS:2 * FS], ys[1][:, :FS], ys[1][:, FS:2 * FS])
        o_early = {k: _dot(y_ops[k], w_ops[k]) for k in (4, 1)}
        _strassen(lambda k: o_early[k] if k in o_early else _dot(y_ops[k], w_ops[k]), put_out)
        return carry

    lax.fori_loop(0, NSTEP, gating_step, 0)
    for i in range(NSTEP):
        for q in range(4):
            for b in range(2):
                o_cp(i, q, b).wait()


@jax.jit
def pallas_adaLN_cond__grouped_kv_mqa__mixer_gmlp__prompt_kernel(
    A_x: jax.Array,
    A_wq: jax.Array,
    A_wk: jax.Array,
    A_wv: jax.Array,
    A_wo: jax.Array,
    B_x: jax.Array,
    B_w_in: jax.Array,
    B_w_sp: jax.Array,
    B_b_sp: jax.Array,
    B_w_out: jax.Array,
    c: jax.Array,
    w_mod: jax.Array,
):
    del B_x
    vm = pltpu.VMEM
    scratch = [
        vm((S, D), bf16), vm((D, D), bf16), vm((D, D), bf16), vm((D, 2 * FH), bf16),
        vm((S, S), bf16), vm((FH, D), bf16), vm((D, 6 * D), bf16),
        vm((8, 6 * D), f32),
        vm((2 * DH, D), bf16),
        vm((7, HD, HD), f32),
        vm((NU, DH, QB), f32),
        vm((3, 8, 16 * 128), f32), vm((3, 8, 16 * 128), f32),
        vm((1, DH, QB), f32),
        vm((4, 8, 128), f32),
        vm((SV0 + NVG * 64, 128), u32),
        vm((NC, DH // 2, KC), u32),
        vm((NVG // 2, 7, 8, 16, 128), f32),
        vm((KC, QB), f32),
        vm((S // RB, H, DH, RB), f32),
        vm((S // RB, H, 8, RB), f32),
        vm((S, QB), f32),
        *[vm((9, RB, HD), f32)] * NSTEP,
        vm((2 * len(MIXED), HD, FS), f32),
        vm((2 * RB + 32, D), f32), vm((2 * RB + 32, D), f32),
        vm((2 * RB + 32, FH), f32), vm((2 * RB + 32, FH), f32),
        vm((S, D), f32),
        vm((S, FH), f32),
        vm((S, FH), f32),
        vm((S, 128), f32),
        vm((S, D), bf16),
        vm((S // 128, 128), bf16), vm((1, 2 * D), bf16),
        pltpu.SemaphoreType.DMA((11,)),
        pltpu.SemaphoreType.DMA((len(X_SPLIT) - 1,)),
        pltpu.SemaphoreType.DMA((8 * NSTEP,)),
    ]
    out = pl.pallas_call(
        _kernel,
        out_shape=jax.ShapeDtypeStruct((S, D), bf16),
        in_specs=[pl.BlockSpec(memory_space=pl.ANY)] * 11,
        out_specs=pl.BlockSpec(memory_space=pl.ANY),
        scratch_shapes=scratch,
        compiler_params=pltpu.CompilerParams(vmem_limit_bytes=110 * 2 ** 20),
    )(A_x.reshape(S, D), A_wq, A_wk.T, A_wv.T, A_wo, B_w_in, B_w_sp, B_b_sp.reshape(S // 128, 128),
      B_w_out, c, w_mod)
    return out.reshape(1, S, D)
```
